```python
import os as _os
_os.environ.setdefault("JAX_PLATFORMS", "cpu")
import jax
import jax.numpy as jnp

def _softmax(x, axis=-1):
    return jax.nn.softmax(x, axis=axis)
def _gelu(x):
    return jax.nn.gelu(x, approximate=True)
def _silu(x):
    return jax.nn.silu(x)
def _sigmoid(x):
    return jax.nn.sigmoid(x)
def _layernorm(x, axis=-1, eps=1e-5):
    m = jnp.mean(x, axis=axis, keepdims=True)
    v = jnp.var(x, axis=axis, keepdims=True)
    return (x - m) / jnp.sqrt(v + eps)
def _scatter_add(tgt, idx, src, axis=0):
    return tgt.at[idx].add(src)
def _segment_sum(src, seg, n):
    return jax.ops.segment_sum(src, seg, n)
class _Rng:
    def __init__(self, key):
        self._k = key
    def _next(self):
        self._k, sub = jax.random.split(self._k)
        return sub
    def normal(self, shape):
        return jax.random.normal(self._next(), shape, dtype=jnp.bfloat16)
    def randint(self, lo, hi, shape):
        return jax.random.randint(self._next(), shape, lo, hi, dtype=jnp.int32)
    def uniform(self, shape, lo=0.0, hi=1.0):
        return jax.random.uniform(self._next(), shape, jnp.bfloat16, lo, hi)
    def permutation(self, n):
        return jax.random.permutation(self._next(), n)


kernel_name = 'gated_mix__linear_attn_block__sliding_local_dilated__prompt'

def setup_inputs():
    _rng = _Rng(jax.random.key(int.from_bytes(__import__("os").urandom(4), "little")))
    _w = (lambda a: (lambda t: t.astype(jnp.bfloat16) if jnp.issubdtype(t.dtype, jnp.floating) else t)(jnp.asarray(a)))
    def _A_setup():
        B, S, D = 1, 2048, 512
        return {
            "x": _w((lambda *s: _rng.normal(s) * 0.05)(B, S, D)),
            "wqkv": _w((lambda *s: _rng.normal(s) * 1.6)(D, 3 * D)),
            "wo": _w((lambda *s: _rng.normal(s) * 0.8)(D, D)),
        }
    _A_in = _A_setup()

    def _B_setup():
        B, S, D = 1, 2048, 512
        return {
            "x": _w((lambda *s: _rng.normal(s) * 0.05)(B, S, D)),
            "wqkv": _w((lambda *s: _rng.normal(s) * 0.8)(D, 3 * D)),
            "wo": _w((lambda *s: _rng.normal(s) * 0.05)(D, D)),
        }
    _B_in = _B_setup()

    return {
        "A_x": _A_in["x"],
        "A_wqkv": _A_in["wqkv"],
        "A_wo": _A_in["wo"],
        "B_x": _B_in["x"],
        "B_wqkv": _B_in["wqkv"],
        "B_wo": _B_in["wo"],
        "gate_w": _w((lambda *s: _rng.normal(s) * 0.05)(512) * 16.0),
    }

def reference(A_x, A_wqkv, A_wo, B_x, B_wqkv, B_wo, gate_w):
    def _A_ref(x, wqkv, wo):
        B, S, D = x.shape
        H = 32; Dh = D // H
        qkv = (lambda x, *d: x.transpose(*d))((x @ wqkv).reshape(B, S, 3, H, Dh), 2, 0, 3, 1, 4)
        q, k, v = qkv[0], qkv[1], qkv[2]
        phi = lambda t: jnp.where(t > 0, t + 1, jnp.exp(t)) + 1e-6
        pq, pk = phi(q), phi(k)
        kv = jnp.einsum("bhsd,bhse->bhde", pk, v)
        z = jnp.einsum("bhsd->bhd", pk)
        num = jnp.einsum("bhqd,bhde->bhqe", pq, kv)
        den = jnp.einsum("bhqd,bhd->bhq", pq, z)[..., None] + 1e-6
        o = num / den
        return (lambda x, *d: x.transpose(*d))(o, 0, 2, 1, 3).reshape(B, S, D) @ wo

    def _B_ref(x, wqkv, wo):
        B, S, D = x.shape
        H = 32; Dh = D // H
        W, dil = 8, 2
        qkv = (lambda x, *d: x.transpose(*d))((x @ wqkv).reshape(B, S, 3, H, Dh), 2, 0, 3, 1, 4)
        q, k, v = qkv[0], qkv[1], qkv[2]
        scale = Dh ** -0.5
        pos = jnp.arange(S)
        off = jnp.arange(W) * dil
        idx = pos[:, None] - off[None, :]
        mask = idx >= 0
        idx_c = jnp.where(mask, idx, 0).reshape(-1)
        kg = k[:, :, idx_c, :].reshape(B, H, S, W, Dh)
        vg = v[:, :, idx_c, :].reshape(B, H, S, W, Dh)
        logits = jnp.einsum("bhsd,bhswd->bhsw", q, kg) * scale
        logits = jnp.where(mask[None, None, :, :], logits, -1e9)
        attn = _softmax(logits, axis=-1)
        o = jnp.einsum("bhsw,bhswd->bhsd", attn, vg)
        return (lambda x, *d: x.transpose(*d))(o, 0, 2, 1, 3).reshape(B, S, D) @ wo

    x = A_x
    g = _sigmoid((x * gate_w).sum(-1, keepdims=True))
    a = _A_ref(x, A_wqkv, A_wo)
    b = _B_ref(x, B_wqkv, B_wo)
    return g * a + (1 - g) * b
```

```python
import functools
import math
import jax
import jax.numpy as jnp
from jax import lax
import jax.experimental.pallas as pl
import jax.experimental.pallas.tpu as pltpu

S, D, H, DH = 2048, 512, 32, 16
W, DIL = 8, 2
TM1 = 512
TM = 256
NT = S // TM
HALO = 16
RB = 8
NRB = TM // RB
OC = 64
NOC = TM // OC
PITCH = 18
F32 = jnp.float32
BF16 = jnp.bfloat16
I32 = jnp.int32
U32 = jnp.uint32
NT_DIMS = (((1,), (1,)), ((), ()))
EXP2_SCALE = (DH ** -0.5) * math.log2(math.e)
XSEG = ((0, TM), (TM, TM1), (TM + TM1, TM1), (TM + 2 * TM1, TM1), (S - TM, TM))


def _phi(t):
    return jnp.where(t > 0, t + 1.0, jnp.exp(t)) + 1e-6


def kernel(x_hbm, awqkv_hbm, awo_hbm, bwqkv_hbm, bwo_hbm, gw_hbm, o_hbm,
           x_v, wk_v, wkT_v, wraw_v, wT_v, t_v, wv_v, wo_v, bwo_v, wout_v, g_v, z_v, zrow_v,
           qkv_v, lhs_v, o_v, zero_v, x32_v, gw_v, gwb_v, sem_x, sem_p, sem_w, sem_o):

    def x_copy(i):
        r, n = XSEG[i]
        return pltpu.make_async_copy(x_hbm.at[pl.ds(r, n), :], x_v.at[pl.ds(r, n), :], sem_x.at[i])

    def p_copy(g):
        if g == 0:
            src = awqkv_hbm.at[:, pl.ds(0, D)]
        else:
            src = bwqkv_hbm.at[:, pl.ds((g - 1) * D, D)]
        return pltpu.make_async_copy(src, wraw_v.at[g], sem_p.at[g])

    wk_copy = pltpu.make_async_copy(awqkv_hbm.at[:, pl.ds(D, D)], wk_v, sem_w.at[0])
    wv_copy = pltpu.make_async_copy(awqkv_hbm.at[:, pl.ds(2 * D, D)], wv_v, sem_w.at[1])
    wo_copy = pltpu.make_async_copy(awo_hbm, wo_v, sem_w.at[2])
    bwo_copy = pltpu.make_async_copy(bwo_hbm, bwo_v, sem_w.at[3])
    gw_copy = pltpu.make_async_copy(gw_hbm, gw_v, sem_w.at[4])

    wk_copy.start()
    x_copy(0).start()

    qkv_v[:, 0:HALO, :] = jnp.zeros((16, HALO, 128), F32)
    zero_v[...] = jnp.zeros_like(zero_v)

    wk_copy.wait()
    for g in range(4):
        x_copy(g + 1).start()
        p_copy(g).start()
    wv_copy.start()
    wo_copy.start()
    bwo_copy.start()
    gw_copy.start()
    wkT_v[...] = pltpu.bitcast(wk_v[...].T, U32)

    def token(val8):
        return pltpu.bitcast(val8, I32) & zero_v[...]

    def after(x, tok):
        if tok is None:
            return x
        return pltpu.bitcast(pltpu.bitcast(x, I32) | tok, F32)

    def half(r, m):
        if isinstance(r, int):
            return r // 2
        return pl.multiple_of(r // 2, m // 2)

    def ldb(ref, r, n, m=None):
        return pltpu.bitcast(ref[pl.ds(half(r, m or n), n // 2), :], BF16)

    def qkv_piece(r0, p):
        xt = ldb(x32_v, r0, TM)
        wT = ldb(wT_v, p * 128, 128)
        res = lax.dot_general(xt, wT, NT_DIMS, preferred_element_type=F32)
        qkv_v[p, pl.ds(HALO + r0, TM), :] = res
        return [res[0:8, :], res[TM // 2:TM // 2 + 8, :]]

    def scatter_rows(tj, val):
        for h in range(H):
            t_v[tj, pl.ds(h * PITCH, DH), :] = val[h * DH:(h + 1) * DH, :]

    def gather_rows(tj, d):
        return t_v[tj, pl.ds(d, H, stride=PITCH), :]

    def k_path(r0, n, init):
        xt = x_v[pl.ds(r0, n), :]
        x32_v[pl.ds(half(r0, TM), n // 2), :] = pltpu.bitcast(xt, U32)
        kT = lax.dot_general(ldb(wkT_v, 0, D), xt, NT_DIMS, preferred_element_type=F32)
        pkT = _phi(kT)
        zp = pkT[:, 0:128]
        for j in range(1, n // 128):
            zp = zp + pkT[:, j * 128:(j + 1) * 128]
        gp = jnp.dot(pkT.astype(BF16), ldb(x32_v, r0, n, TM), preferred_element_type=F32)
        if init:
            z_v[...] = zp
            g_v[...] = gp
        else:
            z_v[...] += zp
            g_v[...] += gp

    def prep_group(g):
        grow = g * D if isinstance(g, int) else pl.multiple_of(g * D, D)
        for j in range(4):
            wt = wraw_v[g, j * 128:(j + 1) * 128, :].T.astype(F32)
            scatter_rows(j, wt)
        for j in range(4):
            for d in range(DH):
                wT_v[pl.ds(half(grow + d * H, H), H // 2), j * 128:(j + 1) * 128] = pltpu.bitcast(
                    gather_rows(j, d).astype(BF16), U32)
        for u in range(4):
            qkv_piece(0, 4 * g + u)

    x_copy(0).wait()
    k_path(0, TM, True)

    def p1(t, c):
        r0 = pl.multiple_of(TM + t * TM1, TM)
        pltpu.make_async_copy(x_hbm.at[pl.ds(0, TM1), :], x_v.at[pl.ds(r0, TM1), :], sem_x.at[t + 1]).wait()
        pltpu.make_async_copy(awqkv_hbm.at[:, pl.ds(0, D)], wraw_v.at[t], sem_p.at[t]).wait()
        k_path(r0, TM1, False)
        prep_group(t)
        return c
    lax.fori_loop(0, 3, p1, 0)

    def permute_rows(src_f32, row0, tbase):
        for j in range(4):
            scatter_rows(tbase + j, src_f32[:, j * 128:(j + 1) * 128])
        for j in range(4):
            for d in range(DH):
                wout_v[pl.ds((row0 + d * H) // 2, H // 2), j * 128:(j + 1) * 128] = pltpu.bitcast(
                    gather_rows(tbase + j, d).astype(BF16), U32)

    def vpu_block(r0, slot, b, first, tokval):
        tok = None if tokval is None else token(tokval)
        rb0 = r0 + b * RB
        base = HALO + rb0
        xg = x_v[pl.ds(rb0, RB), :].astype(F32) * gwb_v[...]
        gl = jnp.sum(xg, axis=1, keepdims=True)
        g = jax.nn.sigmoid(gl)
        pq = [_phi(after(qkv_v[j, pl.ds(base, RB), :], tok)) for j in range(4)]
        den = pq[0] * zrow_v[:, 0:128]
        for j in range(1, 4):
            den = den + pq[j] * zrow_v[:, j * 128:(j + 1) * 128]
        den = den + pltpu.roll(den, 64, 1)
        den = den + pltpu.roll(den, 32, 1)
        ra = g / (den + 1e-6)
        for j in range(4):
            lhs_v[slot, pl.ds(b * RB // 2, RB // 2), j * 128:(j + 1) * 128] = pltpu.bitcast(
                (pq[j] * ra).astype(BF16), U32)
        q = [after(qkv_v[4 + j, pl.ds(base, RB), :], tok) for j in range(4)]
        ss = []
        for w in range(W):
            s = q[0] * qkv_v[8, pl.ds(base - DIL * w, RB), :]
            for j in range(1, 4):
                s = s + q[j] * qkv_v[8 + j, pl.ds(base - DIL * w, RB), :]
            s = s + pltpu.roll(s, 64, 1)
            s = s + pltpu.roll(s, 32, 1)
            if first and b * RB < DIL * w:
                pos = rb0 + lax.broadcasted_iota(jnp.int32, (RB, 128), 0)
                s = jnp.where(pos >= DIL * w, s, -4e9)
            ss.append(s)
        mx = ss[0]
        for w in range(1, W):
            mx = jnp.maximum(mx, ss[w])
        es = [jnp.exp2((s - mx) * EXP2_SCALE) for s in ss]
        l = es[0]
        for w in range(1, W):
            l = l + es[w]
        rbn = (1.0 - g) / l
        for j in range(4):
            o = es[0] * qkv_v[12 + j, pl.ds(base, RB), :]
            for w in range(1, W):
                o = o + es[w] * qkv_v[12 + j, pl.ds(base - DIL * w, RB), :]
            lhs_v[slot, pl.ds(b * RB // 2, RB // 2), D + j * 128: D + (j + 1) * 128] = pltpu.bitcast(
                (o * rbn).astype(BF16), U32)

    def out_chunk(r0, slot, k):
        lhs = pltpu.bitcast(lhs_v[slot, pl.ds(k * OC // 2, OC // 2), :], BF16)
        out = jnp.dot(lhs, ldb(wout_v, 0, 2 * D), preferred_element_type=F32)
        o_v[pl.ds(r0 + k * OC, OC), :] = out.astype(BF16)
        return [out[0:8, j * 128:(j + 1) * 128] for j in range(4)]

    def out_dma(i, r0, n=TM):
        return pltpu.make_async_copy(o_v.at[pl.ds(r0, n), :], o_hbm.at[pl.ds(r0, n), :], sem_o.at[i])

    x_copy(4).wait()
    p_copy(3).wait()
    wv_copy.wait()
    wo_copy.wait()
    bwo_copy.wait()
    gw_copy.wait()
    gwb_v[...] = jnp.broadcast_to(gw_v[...].astype(F32).reshape(1, D), (8, D))
    k_path(S - TM, TM, False)
    prep_group(3)
    rr = lax.broadcasted_iota(jnp.int32, (128, 128), 0) // DH
    cc = lax.broadcasted_iota(jnp.int32, (128, 128), 1) // DH
    bd = rr == cc
    kvs = []
    for j in range(4):
        gj = g_v[j * 128:(j + 1) * 128, :].astype(BF16)
        kv = jnp.dot(gj, wv_v[:, j * 128:(j + 1) * 128], preferred_element_type=F32)
        kvs.append(jnp.where(bd, kv, 0.0).astype(BF16))
    toks = sum([qkv_piece(TM, p) for p in range(2)], [])
    ms = [jnp.dot(kvs[j], wo_v[j * 128:(j + 1) * 128, :], preferred_element_type=F32) for j in range(4)]
    m = jnp.concatenate(ms, axis=0)
    permute_rows(m, 0, 4)
    permute_rows(bwo_v[...].astype(F32), D, 8)
    zs = [z_v[pl.ds(d, H, stride=DH), :] for d in range(DH)]
    zperm = jnp.concatenate(zs, axis=0)
    zrow = jnp.sum(zperm.T, axis=0, keepdims=True)
    zrow_v[...] = jnp.broadcast_to(zrow, (8, D))
    toks += sum([qkv_piece(TM, p) for p in range(2, 16)], [])
    for b in range(NRB):
        vpu_block(0, 0, b, True, toks[max(b - 2, 3)])
    for k in range(NOC):
        out_chunk(0, 0, k)
    out_dma(0, 0).start()

    def tile_body(t, r0, slot):
        toks = sum([qkv_piece(r0 + TM, p) for p in range(16)], [])
        for b in range(NRB):
            vpu_block(r0, slot, b, False, toks[b - 2] if b >= 2 else None)
        outs = sum([out_chunk(r0, slot, k) for k in range(NOC)], [])
        out_dma(t, r0).start()
        return outs

    def p2(t, c):
        tile_body(t, pl.multiple_of(t * TM, TM), 0)
        return c
    lax.fori_loop(1, NT - 2, p2, 0)
    toks = tile_body(NT - 2, (NT - 2) * TM, 0)

    r0 = (NT - 1) * TM
    per = OC // RB
    for k in range(NOC):
        for b in range(k * per, (k + 1) * per):
            i = (b * 3) // 4
            vpu_block(r0, 1, b, False, toks[i])
        toks += out_chunk(r0, 1, k)
        out_dma(NT - 1 + k, r0 + k * OC, OC).start()
    for t in range(NT - 1):
        out_dma(t, t * TM).wait()
    for k in range(NOC):
        out_dma(NT - 1 + k, r0 + k * OC, OC).wait()


@jax.jit
def pallas_gated_mix__linear_attn_block__sliding_local_dilated__prompt_kernel(
    A_x, A_wqkv, A_wo, B_x, B_wqkv, B_wo, gate_w):
    x = A_x.reshape(S, D)
    any_spec = pl.BlockSpec(memory_space=pl.ANY)
    out = pl.pallas_call(
        kernel,
        out_shape=jax.ShapeDtypeStruct((S, D), BF16),
        in_specs=[any_spec] * 6,
        out_specs=any_spec,
        scratch_shapes=[
            pltpu.VMEM((S, D), BF16),
            pltpu.VMEM((D, D), BF16),
            pltpu.VMEM((D // 2, D), U32),
            pltpu.VMEM((4, D, D), BF16),
            pltpu.VMEM((2 * D, D), U32),
            pltpu.VMEM((12, H * PITCH, 128), F32),
            pltpu.VMEM((D, D), BF16),
            pltpu.VMEM((D, D), BF16),
            pltpu.VMEM((D, D), BF16),
            pltpu.VMEM((D, D), U32),
            pltpu.VMEM((D, D), F32),
            pltpu.VMEM((D, 128), F32),
            pltpu.VMEM((8, D), F32),
            pltpu.VMEM((16, HALO + S, 128), F32),
            pltpu.VMEM((2, TM // 2, 2 * D), U32),
            pltpu.VMEM((S, D), BF16),
            pltpu.VMEM((8, 128), I32),
            pltpu.VMEM((S // 2, D), U32),
            pltpu.VMEM((D,), BF16),
            pltpu.VMEM((8, D), F32),
            pltpu.SemaphoreType.DMA((5,)),
            pltpu.SemaphoreType.DMA((4,)),
            pltpu.SemaphoreType.DMA((5,)),
            pltpu.SemaphoreType.DMA((NT - 1 + NOC,)),
        ],
        compiler_params=pltpu.CompilerParams(vmem_limit_bytes=100 * 1024 * 1024),
    )(x, A_wqkv, A_wo, B_wqkv, B_wo, gate_w)
    return out.reshape(1, S, D)
```

```python
import functools
import math
import jax
import jax.numpy as jnp
from jax import lax
import jax.experimental.pallas as pl
import jax.experimental.pallas.tpu as pltpu

S, D, H, DH = 2048, 512, 32, 16
W, DIL = 8, 2
TM1 = 512
TM = 256
NT = S // TM
HALO = 16
RB = 8
NRB = TM // RB
OC = 64
NOC = TM // OC
PITCH = 18
MID_OFF = 3
TAIL_NUM, TAIL_DEN = 1, 1
F32 = jnp.float32
BF16 = jnp.bfloat16
I32 = jnp.int32
U32 = jnp.uint32
NT_DIMS = (((1,), (1,)), ((), ()))
EXP2_SCALE = (DH ** -0.5) * math.log2(math.e)
XSEG = ((0, TM), (TM, TM1), (TM + TM1, TM1), (TM + 2 * TM1, TM1), (S - TM, TM))


def _phi(t):
    return jnp.where(t > 0, t + 1.0, jnp.exp(t)) + 1e-6


def _recip(x):
    x = jnp.minimum(x, 1e38)
    r = pl.reciprocal(x, approx=True)
    return r * (2.0 - x * r)


def kernel(x_hbm, awqkv_hbm, awo_hbm, bwqkv_hbm, bwo_hbm, gw_hbm, o_hbm,
           x_v, wk_v, wkT_v, wraw_v, wT_v, t_v, wv_v, wo_v, bwo_v, wout_v, g_v, z_v, zrow_v,
           qkv_v, lhs_v, o_v, zero_v, x32_v, gw_v, gwb_v, gate_v, xs_v,
           sem_x, sem_p, sem_w, sem_o):

    def x_copy(i):
        r, n = XSEG[i]
        return pltpu.make_async_copy(x_hbm.at[pl.ds(r, n), :], x_v.at[pl.ds(r, n), :], sem_x.at[i])

    def p_copy(g):
        if g == 0:
            src = awqkv_hbm.at[:, pl.ds(0, D)]
        else:
            src = bwqkv_hbm.at[:, pl.ds((g - 1) * D, D)]
        return pltpu.make_async_copy(src, wraw_v.at[g], sem_p.at[g])

    wk_copy = pltpu.make_async_copy(awqkv_hbm.at[:, pl.ds(D, D)], wk_v, sem_w.at[0])
    wv_copy = pltpu.make_async_copy(awqkv_hbm.at[:, pl.ds(2 * D, D)], wv_v, sem_w.at[1])
    wo_copy = pltpu.make_async_copy(awo_hbm, wo_v, sem_w.at[2])
    bwo_copy = pltpu.make_async_copy(bwo_hbm, bwo_v, sem_w.at[3])
    gw_copy = pltpu.make_async_copy(gw_hbm, gw_v, sem_w.at[4])

    gw_copy.start()
    wk_copy.start()
    x_copy(0).start()

    qkv_v[0:16, 0:HALO, :] = jnp.zeros((16, HALO, 128), F32)
    zero_v[...] = jnp.zeros_like(zero_v)

    gw_copy.wait()
    wk_copy.wait()
    for g in range(4):
        x_copy(g + 1).start()
        p_copy(g).start()
    wv_copy.start()
    wo_copy.start()
    bwo_copy.start()
    wkT_v[...] = pltpu.bitcast(wk_v[...].T, U32)
    gwb_v[...] = jnp.broadcast_to(gw_v[...].astype(F32).reshape(1, D), (8, D))

    def token(val8):
        return pltpu.bitcast(val8, I32) & zero_v[...]

    def after(x, tok):
        if tok is None:
            return x
        return pltpu.bitcast(pltpu.bitcast(x, I32) | tok, F32)

    def half(r, m):
        if isinstance(r, int):
            return r // 2
        return pl.multiple_of(r // 2, m // 2)

    def ldb(ref, r, n, m=None):
        return pltpu.bitcast(ref[pl.ds(half(r, m or n), n // 2), :], BF16)

    def put_halos(halos):
        for i, v in halos:
            qkv_v[i, pl.ds(0, HALO), :] = v

    def qkv_piece(xsrc, p, qs, halos=None):
        if xsrc[0] == "x":
            xt = ldb(x32_v, xsrc[1], TM)
        else:
            xt = pltpu.bitcast(xs_v[xsrc[1]], BF16)
        wT = ldb(wT_v, p * 128, 128)
        res = lax.dot_general(xt, wT, NT_DIMS, preferred_element_type=F32)
        qkv_v[16 * qs + p, pl.ds(HALO, TM), :] = res
        if halos is None:
            qkv_v[16 * (1 - qs) + p, pl.ds(0, HALO), :] = res[TM - HALO:TM, :]
        elif p >= 8:
            halos.append((16 * (1 - qs) + p, res[TM - HALO:TM, :]))
        return [res[0:8, :], res[TM // 2:TM // 2 + 8, :]]

    def scatter_rows(tj, val):
        for h in range(H):
            t_v[tj, pl.ds(h * PITCH, DH), :] = val[h * DH:(h + 1) * DH, :]

    def gather_rows(tj, d):
        return t_v[tj, pl.ds(d, H, stride=PITCH), :]

    def gate_rows(r0, n, tokval):
        gwb = gwb_v[...]
        if tokval is not None:
            tok = token(tokval)
            gwb = jnp.concatenate([after(gwb[:, j * 128:(j + 1) * 128], tok) for j in range(4)], axis=1)
        for b in range(n // 8):
            xg = x_v[pl.ds(r0 + b * 8, 8), :].astype(F32) * gwb
            gl = jnp.broadcast_to(jnp.sum(xg, axis=1, keepdims=True), (8, 128))
            gate_v[0, pl.ds(r0 + b * 8, 8), :] = 1.0 + jnp.exp(-gl)
            gate_v[1, pl.ds(r0 + b * 8, 8), :] = 1.0 + jnp.exp(gl)

    def k_path(r0, n, init, gate=True):
        xt = x_v[pl.ds(r0, n), :]
        x32_v[pl.ds(half(r0, TM), n // 2), :] = pltpu.bitcast(xt, U32)
        kT = lax.dot_general(ldb(wkT_v, 0, D), xt, NT_DIMS, preferred_element_type=F32)
        pkT = _phi(kT)
        if gate:
            gate_rows(r0, n, None)
        zp = pkT[:, 0:128]
        for j in range(1, n // 128):
            zp = zp + pkT[:, j * 128:(j + 1) * 128]
        gp = jnp.dot(pkT.astype(BF16), ldb(x32_v, r0, n, TM), preferred_element_type=F32)
        if init:
            z_v[...] = zp
            g_v[...] = gp
        else:
            z_v[...] += zp
            g_v[...] += gp
        nk = n // 128
        if nk == 4:
            return [kT[0:8, 384:512], gp[0:8, 0:128], gp[0:8, 128:256], gp[0:8, 256:384]]
        return [kT[0:8, 0:128], kT[256:264, 0:128], kT[0:8, 128:256], kT[256:264, 128:256]]

    def prep_group(g, tk, npc=4):
        grow = g * D if isinstance(g, int) else pl.multiple_of(g * D, D)
        for j in range(4):
            tok = pltpu.bitcast(token(tk[j]), U32)
            wr = pltpu.bitcast(wraw_v[g, j * 128:(j + 1) * 128, :], U32)
            wr = wr | jnp.tile(tok, (8, 4))
            wt = pltpu.bitcast(wr, BF16).T.astype(F32)
            scatter_rows(j, wt)
        for j in range(4):
            for d in range(DH):
                wT_v[pl.ds(half(grow + d * H, H), H // 2), j * 128:(j + 1) * 128] = pltpu.bitcast(
                    gather_rows(j, d).astype(BF16), U32)
        return sum([qkv_piece(("x", 0), 4 * g + u, 0) for u in range(npc)], [])

    x_copy(0).wait()
    k_path(0, TM, True)

    def p1(t, c):
        r0 = pl.multiple_of(TM + t * TM1, TM)
        pltpu.make_async_copy(x_hbm.at[pl.ds(0, TM1), :], x_v.at[pl.ds(r0, TM1), :], sem_x.at[t + 1]).wait()
        pltpu.make_async_copy(awqkv_hbm.at[:, pl.ds(0, D)], wraw_v.at[t], sem_p.at[t]).wait()
        prep_group(t, k_path(r0, TM1, False))
        return c
    lax.fori_loop(0, 2, p1, 0)

    def permute_rows(src_f32, row0, tbase):
        for j in range(4):
            scatter_rows(tbase + j, src_f32[:, j * 128:(j + 1) * 128])
        for j in range(4):
            for d in range(DH):
                wout_v[pl.ds((row0 + d * H) // 2, H // 2), j * 128:(j + 1) * 128] = pltpu.bitcast(
                    gather_rows(tbase + j, d).astype(BF16), U32)

    def vpu_block(gsrc, slot, b, first, tokval):
        tok = None if tokval is None else token(tokval)
        base = HALO + b * RB
        qb = 16 * slot
        if gsrc[0] == "x":
            ga = gate_v[0, pl.ds(gsrc[1] + b * RB, RB), :]
            gb = gate_v[1, pl.ds(gsrc[1] + b * RB, RB), :]
        else:
            ga = gs_v[2 * gsrc[1], pl.ds(b * RB, RB), :]
            gb = gs_v[2 * gsrc[1] + 1, pl.ds(b * RB, RB), :]
        pq = [_phi(after(qkv_v[qb + j, pl.ds(base, RB), :], tok)) for j in range(4)]
        den = pq[0] * zrow_v[:, 0:128]
        for j in range(1, 4):
            den = den + pq[j] * zrow_v[:, j * 128:(j + 1) * 128]
        den = den + pltpu.roll(den, 64, 1)
        den = den + pltpu.roll(den, 32, 1)
        ra = _recip(ga * (den + 1e-6))
        for j in range(4):
            lhs_v[slot, pl.ds(b * RB // 2, RB // 2), j * 128:(j + 1) * 128] = pltpu.bitcast(
                (pq[j] * ra).astype(BF16), U32)
        q = [after(qkv_v[qb + 4 + j, pl.ds(base, RB), :], tok) for j in range(4)]
        ss = []
        for w in range(W):
            s = q[0] * qkv_v[qb + 8, pl.ds(base - DIL * w, RB), :]
            for j in range(1, 4):
                s = s + q[j] * qkv_v[qb + 8 + j, pl.ds(base - DIL * w, RB), :]
            s = s + pltpu.roll(s, 64, 1)
            s = s + pltpu.roll(s, 32, 1)
            if first and b * RB < DIL * w:
                pos = b * RB + lax.broadcasted_iota(jnp.int32, (RB, 128), 0)
                s = jnp.where(pos >= DIL * w, s, -4e9)
            ss.append(s)
        mx = ss[0]
        for w in range(1, W):
            mx = jnp.maximum(mx, ss[w])
        es = [jnp.exp2((s - mx) * EXP2_SCALE) for s in ss]
        l = es[0]
        for w in range(1, W):
            l = l + es[w]
        rbn = _recip(gb * l)
        for j in range(4):
            o = es[0] * qkv_v[qb + 12 + j, pl.ds(base, RB), :]
            for w in range(1, W):
                o = o + es[w] * qkv_v[qb + 12 + j, pl.ds(base - DIL * w, RB), :]
            lhs_v[slot, pl.ds(b * RB // 2, RB // 2), D + j * 128: D + (j + 1) * 128] = pltpu.bitcast(
                (o * rbn).astype(BF16), U32)

    def out_chunk(r0, slot, k):
        lhs = pltpu.bitcast(lhs_v[slot, pl.ds(k * OC // 2, OC // 2), :], BF16)
        out = jnp.dot(lhs, ldb(wout_v, 0, 2 * D), preferred_element_type=F32)
        o_v[pl.ds(r0 + k * OC, OC), :] = out.astype(BF16)
        return [out[0:8, j * 128:(j + 1) * 128] for j in range(4)]

    def out_dma(i, r0, n=TM):
        return pltpu.make_async_copy(o_v.at[pl.ds(r0, n), :], o_hbm.at[pl.ds(r0, n), :], sem_o.at[i])

    def xs_copy(u, r):
        xs_v[u] = x32_v[pl.ds(half(r, TM), TM // 2), :]

    x_copy(3).wait()
    p_copy(2).wait()
    x_copy(4).wait()
    p_copy(3).wait()
    wv_copy.wait()
    wo_copy.wait()
    bwo_copy.wait()
    for u in range(2):
        xs_copy(u, (2 + u) * TM)
    tk2 = prep_group(2, k_path(TM + 2 * TM1, TM1, False, gate=False))
    prep_group(3, k_path(S - TM, TM, False, gate=False), 2)
    rr = lax.broadcasted_iota(jnp.int32, (128, 128), 0) // DH
    cc = lax.broadcasted_iota(jnp.int32, (128, 128), 1) // DH
    bd = rr == cc
    kvs = []
    for j in range(4):
        gj = g_v[j * 128:(j + 1) * 128, :].astype(BF16)
        kv = jnp.dot(gj, wv_v[:, j * 128:(j + 1) * 128], preferred_element_type=F32)
        kvs.append(jnp.where(bd, kv, 0.0).astype(BF16))
    for u in range(2, 4):
        qkv_piece(("x", 0), 12 + u, 0)
    ms = [jnp.dot(kvs[j], wo_v[j * 128:(j + 1) * 128, :], preferred_element_type=F32) for j in range(4)]
    m = jnp.concatenate(ms, axis=0)
    permute_rows(m, 0, 4)
    for j in range(4):
        tok = token(tk2[2 * j])
        bj = bwo_v[:, j * 128:(j + 1) * 128].astype(F32)
        bj = jnp.concatenate([after(bj[r * 8:(r + 1) * 8], tok) for r in range(D // 8)], axis=0)
        scatter_rows(8 + j, bj)
        for d in range(DH):
            wout_v[pl.ds((D + d * H) // 2, H // 2), j * 128:(j + 1) * 128] = pltpu.bitcast(
                gather_rows(8 + j, d).astype(BF16), U32)
    zs = [z_v[pl.ds(d, H, stride=DH), :] for d in range(DH)]
    zperm = jnp.concatenate(zs, axis=0)
    zrow = jnp.sum(zperm.T, axis=0, keepdims=True)
    zrow_v[...] = jnp.broadcast_to(zrow, (8, D))
    halos = []
    toks = sum([qkv_piece(("x", TM), p, 1, halos) for p in range(16)], [])
    per = OC // RB
    for k in range(NOC):
        for b in range(k * per, (k + 1) * per):
            vpu_block(("x", 0), 0, b, True, toks[b + MID_OFF])
        toks += out_chunk(0, 0, k)
    put_halos(halos)
    out_dma(0, 0).start()
    for i in range(12):
        gate_rows(TM + 2 * TM1 + i * 64, 64, toks[32 + 2 + i])

    def tile_body(t, r0, slot, lead, u=None):
        halos = []
        xsrc = ("x", r0 + TM) if u is None else ("s", u)
        gsrc = ("x", r0)
        toks = lead + sum([qkv_piece(xsrc, p, 1 - slot, halos) for p in range(16)], [])
        if u is not None:
            xs_copy(u, r0 + 3 * TM)
        off = len(lead) - 2
        for b in range(NRB):
            vpu_block(gsrc, slot, b, False, toks[b + off] if b + off >= 0 else None)
        put_halos(halos)
        outs = sum([out_chunk(r0, slot, k) for k in range(NOC)], [])
        out_dma(t, r0).start()
        return outs

    def p2(i, c):
        t = 1 + 2 * i
        r0 = pl.multiple_of(t * TM, TM)
        lead = tile_body(t, r0, 1, [], 0)[-2:]
        tile_body(t + 1, r0 + TM, 0, lead, 1)
        return c
    lax.fori_loop(0, 2, p2, 0)
    r5, r6, r7 = (NT - 3) * TM, (NT - 2) * TM, (NT - 1) * TM
    halos = []
    toks = sum([qkv_piece(("x", r6), p, 0, halos) for p in range(16)], [])
    for b in range(NRB):
        vpu_block(("x", r5), 1, b, False, toks[b - 2] if b >= 2 else None)
    put_halos(halos)
    toks = sum([out_chunk(r5, 1, k) for k in range(2)], [])[-2:]
    toks += sum([qkv_piece(("x", r7), p, 1, []) for p in range(16)], [])
    for b in range(NRB):
        vpu_block(("x", r6), 0, b, False, toks[b])
    toks = toks[-1:] + sum([out_chunk(r5, 1, k) for k in range(2, 4)], [])
    out_dma(NT - 3, r5).start()
    toks += sum([out_chunk(r6, 0, k) for k in range(NOC)], [])
    out_dma(NT - 2, r6).start()
    r0 = r7
    for k in range(NOC):
        for b in range(k * per, (k + 1) * per):
            vpu_block(("x", r0), 1, b, False, toks[(b * TAIL_NUM) // TAIL_DEN])
        toks += out_chunk(r0, 1, k)
        out_dma(NT - 1 + k, r0 + k * OC, OC).start()
    for t in range(NT - 1):
        out_dma(t, t * TM).wait()
    for k in range(NOC):
        out_dma(NT - 1 + k, r0 + k * OC, OC).wait()


@jax.jit
def pallas_gated_mix__linear_attn_block__sliding_local_dilated__prompt_kernel(
    A_x, A_wqkv, A_wo, B_x, B_wqkv, B_wo, gate_w):
    x = A_x.reshape(S, D)
    any_spec = pl.BlockSpec(memory_space=pl.ANY)
    out = pl.pallas_call(
        kernel,
        out_shape=jax.ShapeDtypeStruct((S, D), BF16),
        in_specs=[any_spec] * 6,
        out_specs=any_spec,
        scratch_shapes=[
            pltpu.VMEM((S, D), BF16),
            pltpu.VMEM((D, D), BF16),
            pltpu.VMEM((D // 2, D), U32),
            pltpu.VMEM((4, D, D), BF16),
            pltpu.VMEM((2 * D, D), U32),
            pltpu.VMEM((12, H * PITCH, 128), F32),
            pltpu.VMEM((D, D), BF16),
            pltpu.VMEM((D, D), BF16),
            pltpu.VMEM((D, D), BF16),
            pltpu.VMEM((D, D), U32),
            pltpu.VMEM((D, D), F32),
            pltpu.VMEM((D, 128), F32),
            pltpu.VMEM((8, D), F32),
            pltpu.VMEM((32, HALO + TM, 128), F32),
            pltpu.VMEM((2, TM // 2, 2 * D), U32),
            pltpu.VMEM((S, D), BF16),
            pltpu.VMEM((8, 128), I32),
            pltpu.VMEM((S // 2, D), U32),
            pltpu.VMEM((D,), BF16),
            pltpu.VMEM((8, D), F32),
            pltpu.VMEM((2, S, 128), F32),
            pltpu.VMEM((2, TM // 2, D), U32),
            pltpu.SemaphoreType.DMA((5,)),
            pltpu.SemaphoreType.DMA((4,)),
            pltpu.SemaphoreType.DMA((5,)),
            pltpu.SemaphoreType.DMA((NT - 1 + NOC,)),
        ],
        compiler_params=pltpu.CompilerParams(vmem_limit_bytes=100 * 1024 * 1024),
    )(x, A_wqkv, A_wo, B_wqkv, B_wo, gate_w)
    return out.reshape(1, S, D)
```

```python
import math
import jax
import jax.numpy as jnp
from jax import lax
import jax.experimental.pallas as pl
import jax.experimental.pallas.tpu as pltpu

S, D, H, DH = 2048, 512, 32, 16
W, DIL = 8, 2
TM1 = 512
TM = 256
NT = S // TM
HALO = 16
RB = 8
NRB = TM // RB
OC = 64
NOC = TM // OC
PER = OC // RB
PITCH = 18
MID_OFF = 3
NG2 = 3
PACE_NUM, PACE_DEN = 9, 8
F32 = jnp.float32
BF16 = jnp.bfloat16
I32 = jnp.int32
U32 = jnp.uint32
NT_DIMS = (((1,), (1,)), ((), ()))
SCALE = DH ** -0.5
EXP2_SCALE = SCALE * math.log2(math.e)
MASKED = -1e9 / SCALE
XSEG = ((0, TM), (TM, TM1), (TM + TM1, TM1), (TM + 2 * TM1, TM1), (S - TM, TM))


def _phi(t):
    return jnp.where(t > 0, t + 1.0, jnp.exp(t)) + 1e-6


def _recip(x):
    x = jnp.minimum(x, 1e38)
    r = pl.reciprocal(x, approx=True)
    return r * (2.0 - x * r)


def _kernel(x_hbm, awqkv_hbm, awo_hbm, bwqkv_hbm, bwo_hbm, gw_hbm, o_hbm,
            x_v, wk_v, wkT_v, wraw_v, wT_v, t_v, wv_v, wo_v, bwo_v, wout_v, g_v, z_v, zrow_v,
            qkv_v, lhs_v, o_v, zero_v, x32_v, gw_v, gwb_v, gate_v, sem):

    step = pl.program_id(0)
    live = step == 1
    def x_copy(i):
        r, n = XSEG[i]
        return pltpu.make_async_copy(x_hbm.at[pl.ds(r, n), :], x_v.at[pl.ds(r, n), :],
                                     sem.at[(1, 2, 3, 0, 0)[i]])

    def p_copy(g):
        if g == 0:
            src = awqkv_hbm.at[:, pl.ds(0, D)]
        else:
            src = bwqkv_hbm.at[:, pl.ds((g - 1) * D, D)]
        return pltpu.make_async_copy(src, wraw_v.at[g], sem.at[(2, 3, 0, 0)[g]])

    def out_dma(r0, n=TM):
        return pltpu.make_async_copy(o_v.at[pl.ds(r0, n), :], o_hbm.at[pl.ds(r0, n), :], sem.at[1])

    wk_copy = pltpu.make_async_copy(awqkv_hbm.at[:, pl.ds(D, D)], wk_v, sem.at[0])
    wv_copy = pltpu.make_async_copy(awqkv_hbm.at[:, pl.ds(2 * D, D)], wv_v, sem.at[0])
    wo_copy = pltpu.make_async_copy(awo_hbm, wo_v, sem.at[0])
    bwo_copy = pltpu.make_async_copy(bwo_hbm, bwo_v, sem.at[0])
    gw_copy = pltpu.make_async_copy(gw_hbm, gw_v, sem.at[0])

    @pl.when(step == 0)
    def _start():
        gw_copy.start()
        wk_copy.start()
        x_copy(0).start()

        qkv_v[0:16, 0:HALO, :] = jnp.zeros((16, HALO, 128), F32)
        zero_v[...] = jnp.zeros_like(zero_v)


    @pl.when(live)
    def _prologue():
        gw_copy.wait()
        wk_copy.wait()
        for g in range(4):
            x_copy(g + 1).start()
            p_copy(g).start()
        wv_copy.start()
        wo_copy.start()
        bwo_copy.start()
        wkT_v[...] = pltpu.bitcast(wk_v[...].T, U32)
        gwb_v[...] = jnp.broadcast_to(gw_v[...].astype(F32).reshape(1, D), (8, D))


    def token(val8):
        return pltpu.bitcast(val8, I32) & zero_v[...]

    def after(x, tok):
        if tok is None:
            return x
        return pltpu.bitcast(pltpu.bitcast(x, I32) | tok, F32)

    def half(r, m):
        if isinstance(r, int):
            return r // 2
        return pl.multiple_of(r // 2, m // 2)

    def ldb(ref, r, n, m=None):
        return pltpu.bitcast(ref[pl.ds(half(r, m or n), n // 2), :], BF16)

    def put_halos(halos):
        for i, v in halos:
            qkv_v[i, pl.ds(0, HALO), :] = v

    def qkv_piece(r0, p, qs, halos=None):
        xt = ldb(x32_v, r0, TM)
        wT = ldb(wT_v, p * 128, 128)
        res = lax.dot_general(xt, wT, NT_DIMS, preferred_element_type=F32)
        qkv_v[16 * qs + p, pl.ds(HALO, TM), :] = res
        if halos is None:
            qkv_v[16 * (1 - qs) + p, pl.ds(0, HALO), :] = res[TM - HALO:TM, :]
        elif p >= 8:
            halos.append((16 * (1 - qs) + p, res[TM - HALO:TM, :]))
        return [res[0:8, :], res[TM // 2:TM // 2 + 8, :]]

    def scatter_rows(tj, val):
        for h in range(H):
            t_v[tj, pl.ds(h * PITCH, DH), :] = val[h * DH:(h + 1) * DH, :]

    def gather_rows(tj, d):
        return pltpu.bitcast(t_v[tj, pl.ds(d, H, stride=PITCH), :].astype(BF16), U32)

    def gate_rows(r0, n, tokval):
        gwb = gwb_v[...]
        if tokval is not None:
            tok = token(tokval)
            gwb = jnp.concatenate([after(gwb[:, j * 128:(j + 1) * 128], tok) for j in range(4)], axis=1)
        for b in range(n // 8):
            xg = x_v[pl.ds(r0 + b * 8, 8), :].astype(F32) * gwb
            gl = jnp.broadcast_to(jnp.sum(xg, axis=1, keepdims=True), (8, 128))
            gate_v[0, pl.ds(r0 + b * 8, 8), :] = 1.0 + jnp.exp(-gl)
            gate_v[1, pl.ds(r0 + b * 8, 8), :] = 1.0 + jnp.exp(gl)

    def k_path(r0, n, init, gate=True):
        xt = x_v[pl.ds(r0, n), :]
        x32_v[pl.ds(half(r0, TM), n // 2), :] = pltpu.bitcast(xt, U32)
        kT = lax.dot_general(ldb(wkT_v, 0, D), xt, NT_DIMS, preferred_element_type=F32)
        pkT = _phi(kT)
        if gate:
            gate_rows(r0, n, None)
        zp = pkT[:, 0:128]
        for j in range(1, n // 128):
            zp = zp + pkT[:, j * 128:(j + 1) * 128]
        gp = jnp.dot(pkT.astype(BF16), ldb(x32_v, r0, n, TM), preferred_element_type=F32)
        if init:
            z_v[...] = zp
            g_v[...] = gp
        else:
            z_v[...] += zp
            g_v[...] += gp
        if n == TM1:
            return [kT[0:8, 384:512], gp[0:8, 0:128], gp[0:8, 128:256], gp[0:8, 256:384],
                    gp[256:264, 384:512], gp[384:392, 384:512]]
        return [kT[0:8, 0:128], kT[256:264, 0:128], kT[0:8, 128:256], kT[256:264, 128:256]]

    def prep_group(g, tk, npc=4):
        grow = g * D if isinstance(g, int) else pl.multiple_of(g * D, D)
        for j in range(4):
            tok = pltpu.bitcast(token(tk[j]), U32)
            wr = pltpu.bitcast(wraw_v[g, j * 128:(j + 1) * 128, :], U32)
            wr = wr | jnp.tile(tok, (8, 4))
            scatter_rows(j, pltpu.bitcast(wr, BF16).T.astype(F32))
        for j in range(4):
            for d in range(DH):
                wT_v[pl.ds(half(grow + d * H, H), H // 2), j * 128:(j + 1) * 128] = gather_rows(j, d)
        return sum([qkv_piece(0, 4 * g + u, 0) for u in range(npc)], [])

    def vpu_block(r0, slot, b, first, tokval):
        tok = None if tokval is None else token(tokval)
        base = HALO + b * RB
        qb = 16 * slot
        rows = pl.ds(b * RB // 2, RB // 2)
        ga = gate_v[0, pl.ds(r0 + b * RB, RB), :]
        gb = gate_v[1, pl.ds(r0 + b * RB, RB), :]
        pq = [_phi(after(qkv_v[qb + j, pl.ds(base, RB), :], tok)) for j in range(4)]
        den = pq[0] * zrow_v[:, 0:128]
        for j in range(1, 4):
            den = den + pq[j] * zrow_v[:, j * 128:(j + 1) * 128]
        den = den + pltpu.roll(den, 64, 1)
        den = den + pltpu.roll(den, 32, 1)
        ra = _recip(ga * (den + 1e-6))
        for j in range(4):
            lhs_v[slot, rows, j * 128:(j + 1) * 128] = pltpu.bitcast((pq[j] * ra).astype(BF16), U32)
        q = [after(qkv_v[qb + 4 + j, pl.ds(base, RB), :], tok) for j in range(4)]
        ss = []
        for w in range(W):
            s = q[0] * qkv_v[qb + 8, pl.ds(base - DIL * w, RB), :]
            for j in range(1, 4):
                s = s + q[j] * qkv_v[qb + 8 + j, pl.ds(base - DIL * w, RB), :]
            s = s + pltpu.roll(s, 64, 1)
            s = s + pltpu.roll(s, 32, 1)
            if first and b * RB < DIL * w:
                pos = b * RB + lax.broadcasted_iota(jnp.int32, (RB, 128), 0)
                s = jnp.where(pos >= DIL * w, s, MASKED)
            ss.append(s)
        mx = ss[0]
        for w in range(1, W):
            mx = jnp.maximum(mx, ss[w])
        es = [jnp.exp2((s - mx) * EXP2_SCALE) for s in ss]
        l = es[0]
        for w in range(1, W):
            l = l + es[w]
        rbn = _recip(gb * l)
        for j in range(4):
            o = es[0] * qkv_v[qb + 12 + j, pl.ds(base, RB), :]
            for w in range(1, W):
                o = o + es[w] * qkv_v[qb + 12 + j, pl.ds(base - DIL * w, RB), :]
            lhs_v[slot, rows, D + j * 128: D + (j + 1) * 128] = pltpu.bitcast((o * rbn).astype(BF16), U32)

    def out_chunk(r0, slot, k):
        lhs = pltpu.bitcast(lhs_v[slot, pl.ds(k * OC // 2, OC // 2), :], BF16)
        out = jnp.dot(lhs, ldb(wout_v, 0, 2 * D), preferred_element_type=F32)
        o_v[pl.ds(r0 + k * OC, OC), :] = out.astype(BF16)
        return [out[0:8, j * 128:(j + 1) * 128] for j in range(4)]

    @pl.when(live)
    def _a0():
        x_copy(0).wait()
        k_path(0, TM, True)


    def p1(t, c):
        r0 = pl.multiple_of(TM + t * TM1, TM)
        pltpu.make_async_copy(x_hbm.at[pl.ds(0, TM1), :], x_v.at[pl.ds(r0, TM1), :], sem.at[t + 2]).wait()
        pltpu.make_async_copy(awqkv_hbm.at[:, pl.ds(0, D)], wraw_v.at[t], sem.at[t + 2]).wait()
        tk = k_path(r0, TM1, False, gate=False)
        tq = prep_group(t, tk)
        for i, tv in enumerate((tk[4], tk[5], tq[0], tq[1], tq[2], tq[3], tq[4], tq[5])):
            gate_rows(r0 + i * 64, 64, tv)
        return c
    lax.fori_loop(0, 2 * step, p1, 0)

    @pl.when(live)
    def _mid():
        x_copy(3).wait()
        p_copy(2).wait()
        x_copy(4).wait()
        p_copy(3).wait()
        wv_copy.wait()
        wo_copy.wait()
        bwo_copy.wait()
        tk2 = prep_group(2, k_path(TM + 2 * TM1, TM1, False, gate=False))
        prep_group(3, k_path(S - TM, TM, False, gate=False), 2)
        rr = lax.broadcasted_iota(jnp.int32, (128, 128), 0) // DH
        cc = lax.broadcasted_iota(jnp.int32, (128, 128), 1) // DH
        same_head = rr == cc
        kvs = []
        for j in range(4):
            gj = g_v[j * 128:(j + 1) * 128, :].astype(BF16)
            kv = jnp.dot(gj, wv_v[:, j * 128:(j + 1) * 128], preferred_element_type=F32)
            kvs.append(jnp.where(same_head, kv, 0.0).astype(BF16))
        for u in range(2, 4):
            qkv_piece(0, 12 + u, 0)
        m = jnp.concatenate(
            [jnp.dot(kvs[j], wo_v[j * 128:(j + 1) * 128, :], preferred_element_type=F32) for j in range(4)], axis=0)
        for j in range(4):
            scatter_rows(4 + j, m[:, j * 128:(j + 1) * 128])
        for j in range(4):
            for d in range(DH):
                wout_v[pl.ds(d * H // 2, H // 2), j * 128:(j + 1) * 128] = gather_rows(4 + j, d)
        for j in range(4):
            tok = token(tk2[2 * j])
            bj = bwo_v[:, j * 128:(j + 1) * 128].astype(F32)
            bj = jnp.concatenate([after(bj[r * 8:(r + 1) * 8], tok) for r in range(D // 8)], axis=0)
            scatter_rows(8 + j, bj)
            for d in range(DH):
                wout_v[pl.ds((D + d * H) // 2, H // 2), j * 128:(j + 1) * 128] = gather_rows(8 + j, d)
        zperm = jnp.concatenate([z_v[pl.ds(d, H, stride=DH), :] for d in range(DH)], axis=0)
        zrow_v[...] = jnp.broadcast_to(jnp.sum(zperm.T, axis=0, keepdims=True), (8, D))
        halos = []
        toks = sum([qkv_piece(TM, p, 1, halos) for p in range(16)], [])
        for k in range(NOC):
            for b in range(k * PER, (k + 1) * PER):
                vpu_block(0, 0, b, True, toks[b + MID_OFF])
            toks += out_chunk(0, 0, k)
        put_halos(halos)
        out_dma(0).start()
        for i in range(12):
            gate_rows(TM + 2 * TM1 + i * 64, 64, toks[32 + 2 + i])


    def tile_body(r0, slot, lead):
        halos = []
        toks = lead + sum([qkv_piece(r0 + TM, p, 1 - slot, halos) for p in range(16)], [])
        off = len(lead) - 2
        for k in range(NOC):
            for b in range(k * PER, (k + 1) * PER):
                i = off + (b * PACE_NUM) // PACE_DEN
                vpu_block(r0, slot, b, False, toks[i] if i >= 0 else None)
            toks += out_chunk(r0, slot, k)
        put_halos(halos)
        out_dma(r0).start()
        return toks

    def _body(i, c):
        lead = []
        for t in range(1, 1 + NG2):
            lead = tile_body(t * TM, t % 2, lead)[-2:]
        return c
    lax.fori_loop(0, step, _body, 0)

    @pl.when(live)
    def _tail():
        r5, r6, r7 = (NT - 3) * TM, (NT - 2) * TM, (NT - 1) * TM
        lead = []
        for t in range(1 + NG2, NT - 3):
            lead = tile_body(t * TM, t % 2, lead)[-2:]
        halos = []
        toks = lead + sum([qkv_piece(r6, p, 0, halos) for p in range(16)], [])
        off = len(lead) - 2
        for b in range(NRB):
            vpu_block(r5, 1, b, False, toks[b + off] if b + off >= 0 else None)
        put_halos(halos)
        toks = sum([out_chunk(r5, 1, k) for k in range(2)], [])[-2:]
        toks += sum([qkv_piece(r7, p, 1, []) for p in range(16)], [])
        for b in range(NRB):
            vpu_block(r6, 0, b, False, toks[b])
        toks = toks[-1:] + sum([out_chunk(r5, 1, k) for k in range(2, 4)], [])
        out_dma(r5).start()
        toks += sum([out_chunk(r6, 0, k) for k in range(NOC)], [])
        out_dma(r6).start()
        for k in range(NOC):
            for b in range(k * PER, (k + 1) * PER):
                vpu_block(r7, 1, b, False, toks[b])
            toks += out_chunk(r7, 1, k)
            out_dma(r7 + k * OC, OC).start()
        out_dma(0, S).wait()


@jax.jit
def pallas_gated_mix__linear_attn_block__sliding_local_dilated__prompt_kernel(
    A_x: jax.Array,
    A_wqkv: jax.Array,
    A_wo: jax.Array,
    B_x: jax.Array,
    B_wqkv: jax.Array,
    B_wo: jax.Array,
    gate_w: jax.Array,
):
    x = A_x.reshape(S, D)
    any_spec = pl.BlockSpec(memory_space=pl.ANY)
    out = pl.pallas_call(
        _kernel,
        out_shape=jax.ShapeDtypeStruct((S, D), BF16),
        grid=(2,),
        in_specs=[any_spec] * 6,
        out_specs=any_spec,
        scratch_shapes=[
            pltpu.VMEM((S, D), BF16),
            pltpu.VMEM((D, D), BF16),
            pltpu.VMEM((D // 2, D), U32),
            pltpu.VMEM((4, D, D), BF16),
            pltpu.VMEM((2 * D, D), U32),
            pltpu.VMEM((12, H * PITCH, 128), F32),
            pltpu.VMEM((D, D), BF16),
            pltpu.VMEM((D, D), BF16),
            pltpu.VMEM((D, D), BF16),
            pltpu.VMEM((D, D), U32),
            pltpu.VMEM((D, D), F32),
            pltpu.VMEM((D, 128), F32),
            pltpu.VMEM((8, D), F32),
            pltpu.VMEM((32, HALO + TM, 128), F32),
            pltpu.VMEM((2, TM // 2, 2 * D), U32),
            pltpu.VMEM((S, D), BF16),
            pltpu.VMEM((8, 128), I32),
            pltpu.VMEM((S // 2, D), U32),
            pltpu.VMEM((D,), BF16),
            pltpu.VMEM((8, D), F32),
            pltpu.VMEM((2, S, 128), F32),
            pltpu.SemaphoreType.DMA((4,)),
        ],
        compiler_params=pltpu.CompilerParams(vmem_limit_bytes=100 * 1024 * 1024,
                                             dimension_semantics=("arbitrary",)),
    )(x, A_wqkv, A_wo, B_wqkv, B_wo, gate_w)
    return out.reshape(1, S, D)
```

```python
import math
import jax
import jax.numpy as jnp
from jax import lax
import jax.experimental.pallas as pl
import jax.experimental.pallas.tpu as pltpu

S, D, H, DH = 2048, 512, 32, 16
W, DIL = 8, 2
TM1 = 512
TM = 256
NT = S // TM
HALO = 16
RB = 8
NRB = TM // RB
OC = 64
NOC = TM // OC
PER = OC // RB
PITCH = 18
MID_OFF = 3
NG2 = 3
PACE_NUM, PACE_DEN = 9, 8
F32 = jnp.float32
BF16 = jnp.bfloat16
I32 = jnp.int32
U32 = jnp.uint32
NT_DIMS = (((1,), (1,)), ((), ()))
SCALE = DH ** -0.5
EXP2_SCALE = SCALE * math.log2(math.e)
MASKED = -1e9 / SCALE
XSEG = ((0, TM), (TM, TM1), (TM + TM1, TM1), (TM + 2 * TM1, TM1), (S - TM, TM))


def _phi(t):
    return jnp.where(t > 0, t + 1.0, jnp.exp(t)) + 1e-6


def _recip(x):
    x = jnp.minimum(x, 1e38)
    r = pl.reciprocal(x, approx=True)
    return r * (2.0 - x * r)


def _kernel(x_hbm, awqkv_hbm, awo_hbm, bwqkv_hbm, bwo_hbm, gw_hbm, o_hbm,
            x_v, wk_v, wkT_v, wraw_v, wT_v, t_v, wv_v, wo_v, bwo_v, wout_v, g_v, z_v, zrow_v,
            qkv_v, lhs_v, o_v, zero_v, x32_v, gw_v, gwb_v, gate_v, sem):

    step = pl.program_id(0)
    live = step == 1
    def x_copy(i):
        r, n = XSEG[i]
        return pltpu.make_async_copy(x_hbm.at[pl.ds(r, n), :], x_v.at[pl.ds(r, n), :],
                                     sem.at[(1, 2, 3, 0, 0)[i]])

    def p_copy(g):
        if g == 0:
            src = awqkv_hbm.at[:, pl.ds(0, D)]
        else:
            src = bwqkv_hbm.at[:, pl.ds((g - 1) * D, D)]
        return pltpu.make_async_copy(src, wraw_v.at[g], sem.at[(2, 3, 0, 0)[g]])

    def out_dma(r0, n=TM):
        return pltpu.make_async_copy(o_v.at[pl.ds(r0, n), :], o_hbm.at[pl.ds(r0, n), :], sem.at[1])

    wk_copy = pltpu.make_async_copy(awqkv_hbm.at[:, pl.ds(D, D)], wk_v, sem.at[0])
    wv_copy = pltpu.make_async_copy(awqkv_hbm.at[:, pl.ds(2 * D, D)], wv_v, sem.at[0])
    wo_copy = pltpu.make_async_copy(awo_hbm, wo_v, sem.at[0])
    bwo_copy = pltpu.make_async_copy(bwo_hbm, bwo_v, sem.at[0])
    gw_copy = pltpu.make_async_copy(gw_hbm, gw_v, sem.at[0])

    @pl.when(step == 0)
    def _start():
        gw_copy.start()
        wk_copy.start()
        x_copy(0).start()

        qkv_v[0:16, 0:HALO, :] = jnp.zeros((16, HALO, 128), F32)
        zero_v[...] = jnp.zeros_like(zero_v)

    @pl.when(live)
    def _prologue():
        gw_copy.wait()
        wk_copy.wait()
        for g in range(4):
            x_copy(g + 1).start()
            p_copy(g).start()
        wv_copy.start()
        wo_copy.start()
        bwo_copy.start()
        wkT_v[...] = pltpu.bitcast(wk_v[...].T, U32)
        gwb_v[...] = jnp.broadcast_to(gw_v[...].astype(F32).reshape(1, D), (8, D))

    def token(val8):
        return pltpu.bitcast(val8, I32) & zero_v[...]

    def after(x, tok):
        if tok is None:
            return x
        return pltpu.bitcast(pltpu.bitcast(x, I32) | tok, F32)

    def half(r, m):
        if isinstance(r, int):
            return r // 2
        return pl.multiple_of(r // 2, m // 2)

    def ldb(ref, r, n, m=None):
        return pltpu.bitcast(ref[pl.ds(half(r, m or n), n // 2), :], BF16)

    def put_halos(halos):
        for i, v in halos:
            qkv_v[i, pl.ds(0, HALO), :] = v

    def qkv_piece(r0, p, qs, halos=None):
        xt = ldb(x32_v, r0, TM)
        wT = ldb(wT_v, p * 128, 128)
        res = lax.dot_general(xt, wT, NT_DIMS, preferred_element_type=F32)
        qkv_v[16 * qs + p, pl.ds(HALO, TM), :] = res
        if halos is None:
            qkv_v[16 * (1 - qs) + p, pl.ds(0, HALO), :] = res[TM - HALO:TM, :]
        elif p >= 8:
            halos.append((16 * (1 - qs) + p, res[TM - HALO:TM, :]))
        return [res[0:8, :], res[TM // 2:TM // 2 + 8, :]]

    def scatter_rows(tj, val):
        for h in range(H):
            t_v[tj, pl.ds(h * PITCH, DH), :] = val[h * DH:(h + 1) * DH, :]

    def gather_rows(tj, d):
        return pltpu.bitcast(t_v[tj, pl.ds(d, H, stride=PITCH), :].astype(BF16), U32)

    def gate_rows(r0, n, tokval):
        gwb = gwb_v[...]
        if tokval is not None:
            tok = token(tokval)
            gwb = jnp.concatenate([after(gwb[:, j * 128:(j + 1) * 128], tok) for j in range(4)], axis=1)
        for b in range(n // 8):
            xg = x_v[pl.ds(r0 + b * 8, 8), :].astype(F32) * gwb
            gl = jnp.broadcast_to(jnp.sum(xg, axis=1, keepdims=True), (8, 128))
            gate_v[0, pl.ds(r0 + b * 8, 8), :] = 1.0 + jnp.exp(-gl)
            gate_v[1, pl.ds(r0 + b * 8, 8), :] = 1.0 + jnp.exp(gl)

    def k_path(r0, n, init, gate=True):
        xt = x_v[pl.ds(r0, n), :]
        x32_v[pl.ds(half(r0, TM), n // 2), :] = pltpu.bitcast(xt, U32)
        kT = lax.dot_general(ldb(wkT_v, 0, D), xt, NT_DIMS, preferred_element_type=F32)
        pkT = _phi(kT)
        if gate:
            gate_rows(r0, n, None)
        zp = pkT[:, 0:128]
        for j in range(1, n // 128):
            zp = zp + pkT[:, j * 128:(j + 1) * 128]
        gp = jnp.dot(pkT.astype(BF16), ldb(x32_v, r0, n, TM), preferred_element_type=F32)
        if init:
            z_v[...] = zp
            g_v[...] = gp
        else:
            z_v[...] += zp
            g_v[...] += gp
        if n == TM1:
            return [kT[0:8, 384:512], gp[0:8, 0:128], gp[0:8, 128:256], gp[0:8, 256:384],
                    gp[256:264, 384:512], gp[384:392, 384:512]]
        return [kT[0:8, 0:128], kT[256:264, 0:128], kT[0:8, 128:256], kT[256:264, 128:256]]

    def prep_group(g, tk, npc=4):
        grow = g * D if isinstance(g, int) else pl.multiple_of(g * D, D)
        for j in range(4):
            tok = pltpu.bitcast(token(tk[j]), U32)
            wr = pltpu.bitcast(wraw_v[g, j * 128:(j + 1) * 128, :], U32)
            wr = wr | jnp.tile(tok, (8, 4))
            scatter_rows(j, pltpu.bitcast(wr, BF16).T.astype(F32))
        for j in range(4):
            for d in range(DH):
                wT_v[pl.ds(half(grow + d * H, H), H // 2), j * 128:(j + 1) * 128] = gather_rows(j, d)
        return sum([qkv_piece(0, 4 * g + u, 0) for u in range(npc)], [])

    def vpu_block(r0, slot, b, first, tokval):
        base = HALO + b * RB
        qb = 16 * slot
        rows = pl.ds(b * RB // 2, RB // 2)
        ga = gate_v[0, pl.ds(r0 + b * RB, RB), :]
        gb = gate_v[1, pl.ds(r0 + b * RB, RB), :]
        qq = qkv_v[qb:qb + 8, pl.ds(base, RB), :]
        if tokval is not None:
            qq = lax.bitcast_convert_type(
                lax.bitcast_convert_type(qq, I32) | token(tokval)[None], F32)
        pq = _phi(qq[0:4])
        den = jnp.sum(pq * zrow_v[...], axis=0)
        den = den + pltpu.roll(den, 64, 1)
        den = den + pltpu.roll(den, 32, 1)
        ra = _recip(ga * (den + 1e-6))
        lhs_v[8 * slot:8 * slot + 4, rows, :] = pltpu.bitcast((pq * ra[None]).astype(BF16), U32)
        q = qq[4:8]
        s = jnp.concatenate(
            [jnp.sum(q * qkv_v[qb + 8:qb + 12, pl.ds(base - DIL * w, RB), :], axis=0) for w in range(W)],
            axis=0)
        s = s + pltpu.roll(s, 64, 1)
        s = s + pltpu.roll(s, 32, 1)
        s = s.reshape(W, RB, 128)
        if first and b * RB < DIL * (W - 1):
            pos = b * RB + lax.broadcasted_iota(jnp.int32, (W, RB, 128), 1)
            off = DIL * lax.broadcasted_iota(jnp.int32, (W, RB, 128), 0)
            s = jnp.where(pos >= off, s, MASKED)
        mx = s[0]
        for w in range(1, W):
            mx = jnp.maximum(mx, s[w])
        es = jnp.exp2((s - mx[None]) * EXP2_SCALE)
        l = es[0]
        for w in range(1, W):
            l = l + es[w]
        rbn = _recip(gb * l)
        o = es[0][None] * qkv_v[qb + 12:qb + 16, pl.ds(base, RB), :]
        for w in range(1, W):
            o = o + es[w][None] * qkv_v[qb + 12:qb + 16, pl.ds(base - DIL * w, RB), :]
        lhs_v[8 * slot + 4:8 * slot + 8, rows, :] = pltpu.bitcast((o * rbn[None]).astype(BF16), U32)

    def out_chunk(r0, slot, k):
        lhs = jnp.concatenate(
            [lhs_v[8 * slot + j, pl.ds(k * OC // 2, OC // 2), :] for j in range(8)], axis=1)
        out = jnp.dot(pltpu.bitcast(lhs, BF16), ldb(wout_v, 0, 2 * D), preferred_element_type=F32)
        o_v[pl.ds(r0 + k * OC, OC), :] = out.astype(BF16)
        return [out[0:8, j * 128:(j + 1) * 128] for j in range(4)]

    def out_wide(r0, slot, k2):
        lhs = jnp.concatenate(
            [lhs_v[8 * slot + j, pl.ds(k2 * OC, OC), :] for j in range(8)], axis=1)
        out = jnp.dot(pltpu.bitcast(lhs, BF16), ldb(wout_v, 0, 2 * D), preferred_element_type=F32)
        o_v[pl.ds(r0 + k2 * 2 * OC, 2 * OC), :] = out.astype(BF16)
        return sum([[out[0:8, j * 128:(j + 1) * 128], out[2 * OC - 8:2 * OC, j * 128:(j + 1) * 128]]
                    for j in range(4)], [])

    @pl.when(live)
    def _a0():
        x_copy(0).wait()
        k_path(0, TM, True)

    def p1(t, c):
        r0 = pl.multiple_of(TM + t * TM1, TM)
        pltpu.make_async_copy(x_hbm.at[pl.ds(0, TM1), :], x_v.at[pl.ds(r0, TM1), :], sem.at[t + 2]).wait()
        pltpu.make_async_copy(awqkv_hbm.at[:, pl.ds(0, D)], wraw_v.at[t], sem.at[t + 2]).wait()
        tk = k_path(r0, TM1, False, gate=False)
        tq = prep_group(t, tk)
        for i, tv in enumerate((tk[4], tk[5], tq[0], tq[1], tq[2], tq[3], tq[4], tq[5])):
            gate_rows(r0 + i * 64, 64, tv)
        return c
    lax.fori_loop(0, 2 * step, p1, 0)

    @pl.when(live)
    def _mid():
        x_copy(3).wait()
        p_copy(2).wait()
        x_copy(4).wait()
        p_copy(3).wait()
        wv_copy.wait()
        wo_copy.wait()
        bwo_copy.wait()
        tk2 = prep_group(2, k_path(TM + 2 * TM1, TM1, False, gate=False))
        prep_group(3, k_path(S - TM, TM, False, gate=False), 2)
        rr = lax.broadcasted_iota(jnp.int32, (128, 128), 0) // DH
        cc = lax.broadcasted_iota(jnp.int32, (128, 128), 1) // DH
        same_head = rr == cc
        kvs = []
        for j in range(4):
            gj = g_v[j * 128:(j + 1) * 128, :].astype(BF16)
            kv = jnp.dot(gj, wv_v[:, j * 128:(j + 1) * 128], preferred_element_type=F32)
            kvs.append(jnp.where(same_head, kv, 0.0).astype(BF16))
        for u in range(2, 4):
            qkv_piece(0, 12 + u, 0)
        m = jnp.concatenate(
            [jnp.dot(kvs[j], wo_v[j * 128:(j + 1) * 128, :], preferred_element_type=F32) for j in range(4)], axis=0)
        for j in range(4):
            scatter_rows(4 + j, m[:, j * 128:(j + 1) * 128])
        for j in range(4):
            for d in range(DH):
                wout_v[pl.ds(d * H // 2, H // 2), j * 128:(j + 1) * 128] = gather_rows(4 + j, d)
        for j in range(4):
            tok = token(tk2[2 * j])
            bj = bwo_v[:, j * 128:(j + 1) * 128].astype(F32)
            bj = jnp.concatenate([after(bj[r * 8:(r + 1) * 8], tok) for r in range(D // 8)], axis=0)
            scatter_rows(8 + j, bj)
            for d in range(DH):
                wout_v[pl.ds((D + d * H) // 2, H // 2), j * 128:(j + 1) * 128] = gather_rows(8 + j, d)
        zperm = jnp.concatenate([z_v[pl.ds(d, H, stride=DH), :] for d in range(DH)], axis=0)
        zrow = jnp.broadcast_to(jnp.sum(zperm.T, axis=0, keepdims=True), (8, D))
        for j in range(4):
            zrow_v[j] = zrow[:, j * 128:(j + 1) * 128]
        halos = []
        toks = sum([qkv_piece(TM, p, 1, halos) for p in range(16)], [])
        for k in range(NOC):
            for b in range(k * PER, (k + 1) * PER):
                vpu_block(0, 0, b, True, toks[b + MID_OFF])
            toks += out_chunk(0, 0, k)
        put_halos(halos)
        out_dma(0).start()
        for i in range(12):
            gate_rows(TM + 2 * TM1 + i * 64, 64, toks[32 + 2 + i])

    def tile_body(r0, slot, lead):
        halos = []
        toks = lead + sum([qkv_piece(r0 + TM, p, 1 - slot, halos) for p in range(16)], [])
        off = len(lead) - 2
        for k in range(NOC):
            for b in range(k * PER, (k + 1) * PER):
                i = off + (b * PACE_NUM) // PACE_DEN
                vpu_block(r0, slot, b, False, toks[i] if i >= 0 else None)
            toks += out_chunk(r0, slot, k)
        put_halos(halos)
        out_dma(r0).start()
        return toks

    def _body(i, c):
        lead = []
        for t in range(1, 1 + NG2):
            lead = tile_body(t * TM, t % 2, lead)[-2:]
        return c
    lax.fori_loop(0, step, _body, 0)

    @pl.when(live)
    def _tail():
        r5, r6, r7 = (NT - 3) * TM, (NT - 2) * TM, (NT - 1) * TM
        lead = []
        for t in range(1 + NG2, NT - 3):
            lead = tile_body(t * TM, t % 2, lead)[-2:]
        halos = []
        toks = lead + sum([qkv_piece(r6, p, 0, halos) for p in range(16)], [])
        off = len(lead) - 2
        for b in range(NRB):
            vpu_block(r5, 1, b, False, toks[b + off] if b + off >= 0 else None)
        put_halos(halos)
        toks = sum([out_chunk(r5, 1, k) for k in range(2)], [])[-2:]
        toks += sum([qkv_piece(r7, p, 1, []) for p in range(16)], [])
        for b in range(NRB):
            vpu_block(r6, 0, b, False, toks[b])
        toks = toks[-2:] + out_wide(r5, 1, 1)
        out_dma(r5).start()
        toks += out_wide(r6, 0, 0) + out_wide(r6, 0, 1)
        out_dma(r6).start()
        for k in range(NOC):
            for b in range(k * PER, (k + 1) * PER):
                vpu_block(r7, 1, b, False, toks[b])
            toks += out_chunk(r7, 1, k)
            out_dma(r7 + k * OC, OC).start()
        out_dma(0, S).wait()


@jax.jit
def pallas_gated_mix__linear_attn_block__sliding_local_dilated__prompt_kernel(
    A_x: jax.Array,
    A_wqkv: jax.Array,
    A_wo: jax.Array,
    B_x: jax.Array,
    B_wqkv: jax.Array,
    B_wo: jax.Array,
    gate_w: jax.Array,
):
    x = A_x.reshape(S, D)
    any_spec = pl.BlockSpec(memory_space=pl.ANY)
    out = pl.pallas_call(
        _kernel,
        out_shape=jax.ShapeDtypeStruct((S, D), BF16),
        grid=(2,),
        in_specs=[any_spec] * 6,
        out_specs=any_spec,
        scratch_shapes=[
            pltpu.VMEM((S, D), BF16),
            pltpu.VMEM((D, D), BF16),
            pltpu.VMEM((D // 2, D), U32),
            pltpu.VMEM((4, D, D), BF16),
            pltpu.VMEM((2 * D, D), U32),
            pltpu.VMEM((12, H * PITCH, 128), F32),
            pltpu.VMEM((D, D), BF16),
            pltpu.VMEM((D, D), BF16),
            pltpu.VMEM((D, D), BF16),
            pltpu.VMEM((D, D), U32),
            pltpu.VMEM((D, D), F32),
            pltpu.VMEM((D, 128), F32),
            pltpu.VMEM((4, 8, 128), F32),
            pltpu.VMEM((32, HALO + TM, 128), F32),
            pltpu.VMEM((16, TM // 2, 128), U32),
            pltpu.VMEM((S, D), BF16),
            pltpu.VMEM((8, 128), I32),
            pltpu.VMEM((S // 2, D), U32),
            pltpu.VMEM((D,), BF16),
            pltpu.VMEM((8, D), F32),
            pltpu.VMEM((2, S, 128), F32),
            pltpu.SemaphoreType.DMA((4,)),
        ],
        compiler_params=pltpu.CompilerParams(vmem_limit_bytes=100 * 1024 * 1024,
                                             dimension_semantics=("arbitrary",)),
    )(x, A_wqkv, A_wo, B_wqkv, B_wo, gate_w)
    return out.reshape(1, S, D)
```
